```python
import jax
import jax.numpy as jnp

def _softmax(x, axis=-1):
    return jax.nn.softmax(x, axis=axis)
def _gelu(x):
    return jax.nn.gelu(x, approximate=True)
def _silu(x):
    return jax.nn.silu(x)
def _sigmoid(x):
    return jax.nn.sigmoid(x)
def _layernorm(x, axis=-1, eps=1e-5):
    m = jnp.mean(x, axis=axis, keepdims=True)
    v = jnp.var(x, axis=axis, keepdims=True)
    return (x - m) / jnp.sqrt(v + eps)
def _scatter_add(tgt, idx, src, axis=0):
    return tgt.at[idx].add(src)
def _segment_sum(src, seg, n):
    return jax.ops.segment_sum(src, seg, n)
class _Rng:
    def __init__(self, key):
        self._k = key
    def _next(self):
        self._k, sub = jax.random.split(self._k)
        return sub
    def normal(self, shape):
        return jax.random.normal(self._next(), shape, dtype=jnp.bfloat16)
    def randint(self, lo, hi, shape):
        return jax.random.randint(self._next(), shape, lo, hi, dtype=jnp.int32)
    def uniform(self, shape, lo=0.0, hi=1.0):
        return jax.random.uniform(self._next(), shape, jnp.bfloat16, lo, hi)
    def permutation(self, n):
        return jax.random.permutation(self._next(), n)


kernel_name = 'standalone__groupnorm__prompt'

def setup_inputs():
    _rng = _Rng(jax.random.key(int.from_bytes(__import__("os").urandom(4), "little")))
    _w = (lambda a: (lambda t: t.astype(jnp.bfloat16) if jnp.issubdtype(t.dtype, jnp.floating) else t)(jnp.asarray(a)))
    B = 2
    G = 32
    cpg = max(1, 1024 // G)
    C = G * cpg
    H, W = 32, 2048
    return {
        "x": _w((lambda *s: _rng.normal(s) * 0.05)(B, C, H, W)),
        "g": _w((lambda *s: _rng.normal(s) * 0.05)(C) + 1.0),
        "b": _w((lambda *s: _rng.normal(s) * 0.05)(C)),
    }

def reference(x, g, b):
    G = 32
    B, C, H, W = x.shape[0], x.shape[1], x.shape[2], x.shape[3]
    xr = x.reshape(B, G, C // G, H, W)
    mu = xr.mean(axis=(2, 3, 4), keepdims=True)
    var = ((xr - mu) ** 2).mean(axis=(2, 3, 4), keepdims=True)
    xn = (xr - mu) / jnp.sqrt(var + 1e-5)
    xn = xn.reshape(B, C, H, W)
    return xn * g[None, :, None, None] + b[None, :, None, None]
```

```python
import functools

import jax
import jax.numpy as jnp
from jax import lax
import jax.experimental.pallas as pl
import jax.experimental.pallas.tpu as pltpu

_GROUPS = 32
_EPS = 1e-5
_LANES = 128
_ROWS = 8
_WRITE_WAYS = 4
_WRITE_COLS = 1024
_VMEM_BUDGET = 96 * 2**20


def _phase_sizes(n_groups, max_slots):
    n_phases = -(-n_groups // max_slots)
    base, extra = divmod(n_groups, n_phases)
    return [base + (p < extra) for p in range(n_phases)]


def _lane_splat_table(v_ref, table_ref):
    n = v_ref.shape[0]
    v = v_ref[...].astype(jnp.float32).reshape(1, n)
    for r in range(n // _LANES):
        part = v[:, r * _LANES:(r + 1) * _LANES]
        table_ref[r * _LANES:(r + 1) * _LANES, :] = jnp.broadcast_to(
            part, (_LANES, _LANES)).T


def _all_sum(acc):
    return jnp.sum(jnp.sum(acc, axis=0, keepdims=True), axis=1, keepdims=True)


def _kernel(x_hbm, g_ref, b_ref, o_hbm, buf, g_tab, b_tab, rsem, wsem, *, phases):
    _, ways, cpw, h, w = x_hbm.shape
    cpg = ways * cpw
    inv_n = 1.0 / (cpg * h * w)
    acc_w = min(w, 1024)

    def read(group, slot):
        return pltpu.make_async_copy(x_hbm.at[group], buf.at[slot], rsem.at[slot])

    def start_write(group, slot):
        def per_channel(c, carry):
            for r in range(0, h, _ROWS):
                for l in range(0, w, _WRITE_COLS):
                    rows, cols = pl.ds(r, _ROWS), pl.ds(l, _WRITE_COLS)
                    pltpu.make_async_copy(
                        buf.at[slot, :, c, rows, cols],
                        o_hbm.at[group, :, c, rows, cols],
                        wsem.at[slot]).start()
            return carry
        lax.fori_loop(0, cpw, per_channel, None)

    def wait_write(group, slot):
        pltpu.make_async_copy(buf.at[slot], o_hbm.at[group], wsem.at[slot]).wait()

    def reduce_slot(slot, fn):
        def per_channel(c, acc):
            for r in range(0, h, _ROWS):
                for l in range(0, w, acc_w):
                    v = buf[slot, c // cpw, c % cpw, r:r + _ROWS, l:l + acc_w]
                    acc = acc + fn(v.astype(jnp.float32))
            return acc
        acc = lax.fori_loop(0, cpg, per_channel, jnp.zeros((_ROWS, acc_w), jnp.float32))
        return _all_sum(acc) * inv_n

    def normalise(group, slot):
        mean = jnp.broadcast_to(reduce_slot(slot, lambda v: v), (_ROWS, acc_w))
        var = reduce_slot(slot, lambda v: jnp.square(v - mean))
        rstd = jnp.broadcast_to(lax.rsqrt(var + _EPS), (1, _LANES))
        c0 = (group % _GROUPS) * cpg

        def per_channel(c, carry):
            scale = g_tab[pl.ds(c0 + c, 1), :] * rstd
            shift = b_tab[pl.ds(c0 + c, 1), :]
            scale = jnp.tile(jnp.broadcast_to(scale, (_ROWS, _LANES)), (1, acc_w // _LANES))
            shift = jnp.tile(jnp.broadcast_to(shift, (_ROWS, _LANES)), (1, acc_w // _LANES))
            for r in range(0, h, _ROWS):
                for l in range(0, w, acc_w):
                    idx = (slot, c // cpw, c % cpw, pl.ds(r, _ROWS), pl.ds(l, acc_w))
                    v = buf[idx].astype(jnp.float32)
                    buf[idx] = ((v - mean) * scale + shift).astype(buf.dtype)
            return carry
        lax.fori_loop(0, cpg, per_channel, None)

    def loop(lo, hi, fn):
        if hi > lo:
            lax.fori_loop(lo, hi, lambda i, carry: fn(i), None)

    loop(0, phases[0], lambda s: read(s, s).start())
    _lane_splat_table(g_ref, g_tab)
    _lane_splat_table(b_ref, b_tab)

    first = 0
    for p, size in enumerate(phases):
        nxt_first = first + size
        nxt_size = phases[p + 1] if p + 1 < len(phases) else 0

        def step(s, first=first, size=size):
            read(first + s, s).wait()

            @pl.when(s == size - 1)
            def _():
                loop(0, min(1, size - 1), lambda t: start_write(first + t, t))

            normalise(first + s, s)

        loop(0, size, step)
        loop(min(1, size - 1), size, lambda s: start_write(first + s, s))
        loop(0, size, lambda s: wait_write(first + s, s))
        loop(0, nxt_size, lambda s: read(nxt_first + s, s).start())
        first = nxt_first


@jax.jit
def pallas_standalone__groupnorm__prompt_kernel(
    x: jax.Array,
    g: jax.Array,
    b: jax.Array,
):
    batch, channels, h, w = x.shape
    cpg = channels // _GROUPS
    n_groups = batch * _GROUPS
    group_shape = (_WRITE_WAYS, cpg // _WRITE_WAYS, h, w)
    group_bytes = cpg * h * w * x.dtype.itemsize
    phases = _phase_sizes(n_groups, _VMEM_BUDGET // group_bytes)
    slots = max(phases)

    out = pl.pallas_call(
        functools.partial(_kernel, phases=phases),
        in_specs=[
            pl.BlockSpec(memory_space=pl.ANY),
            pl.BlockSpec(memory_space=pltpu.VMEM),
            pl.BlockSpec(memory_space=pltpu.VMEM),
        ],
        out_specs=pl.BlockSpec(memory_space=pl.ANY),
        out_shape=jax.ShapeDtypeStruct((n_groups, *group_shape), x.dtype),
        scratch_shapes=[
            pltpu.VMEM((slots, *group_shape), x.dtype),
            pltpu.VMEM((channels, _LANES), jnp.float32),
            pltpu.VMEM((channels, _LANES), jnp.float32),
            pltpu.SemaphoreType.DMA((slots,)),
            pltpu.SemaphoreType.DMA((slots,)),
        ],
        compiler_params=pltpu.CompilerParams(vmem_limit_bytes=120 * 2**20),
        name="groupnorm",
    )(x.reshape(n_groups, *group_shape), g, b)
    return out.reshape(x.shape)
```

```python
import functools

import jax
import jax.numpy as jnp
from jax import lax
import jax.experimental.pallas as pl
import jax.experimental.pallas.tpu as pltpu

_GROUPS = 32
_EPS = 1e-5
_LANES = 128
_ROWS = 8
_WAYS = 8
_GROUPS_PER_WINDOW = 2
_READ_COLS = 256
_WRITE_COLS = 1024
_COMPUTE_COLS = 1024
_TAIL_STRIPS = 2
_PHASES = 3


def _loop(lo, hi, fn):
    lax.fori_loop(lo, hi, lambda i, carry: fn(i), None)


def _lane_splat_table(v_ref, table_ref):
    n = v_ref.shape[0]
    v = v_ref[...].astype(jnp.float32).reshape(1, n)
    for c in range(0, n, _LANES):
        table_ref[c:c + _LANES, :] = jnp.broadcast_to(
            v[:, c:c + _LANES], (_LANES, _LANES)).T


def _splat(v):
    return jnp.tile(jnp.broadcast_to(v, (_ROWS, _LANES)), (1, _COMPUTE_COLS // _LANES))


def _kernel(x_hbm, g_hbm, b_hbm, o_hbm, buf, g_vmem, b_vmem, g_tab, b_tab,
            read_sems, tail_sem, write_sems, param_sems, *, height):
    windows, _, strips, _, width = x_hbm.shape
    ways_per_group = _WAYS // _GROUPS_PER_WINDOW
    strips_per_channel = height // _ROWS
    channels_per_way = strips // strips_per_channel
    channels_per_group = ways_per_group * channels_per_way
    inv_count = 1.0 / (channels_per_group * height * width)

    def start_reads(window, slot, lo, hi, sem):
        def strip(s):
            for col in range(0, width, _READ_COLS):
                for thread in range(2):
                    part = (slice(None), s, slice(None), pl.ds(col, _READ_COLS))
                    pltpu.make_async_copy(
                        x_hbm.at[(window + thread, *part)],
                        buf.at[(slot + thread, *part)], sem).start(priority=thread)
        _loop(lo, hi, strip)

    def wait_reads(window, slot, lo, hi, sem):
        part = (slice(None), pl.ds(lo, hi - lo))
        pltpu.make_async_copy(
            x_hbm.at[(pl.ds(window, 2), *part)],
            buf.at[(pl.ds(slot, 2), *part)], sem).wait()

    def start_writes(window, slot):
        def strip(s):
            for col in range(0, width, _WRITE_COLS):
                part = (slice(None), s, slice(None), pl.ds(col, _WRITE_COLS))
                pltpu.make_async_copy(
                    buf.at[(slot, *part)], o_hbm.at[(window, *part)],
                    write_sems.at[slot]).start()
        _loop(0, strips, strip)

    def wait_writes(window, slot):
        pltpu.make_async_copy(
            buf.at[slot], o_hbm.at[window], write_sems.at[slot]).wait()

    def normalise(window, slot, before_pass=lambda i: None):
        def group(k):
            def for_channels(fn, init=None):
                def way(a, carry):
                    def channel(c, carry):
                        tiles = [
                            (slot, k * ways_per_group + a, c * strips_per_channel + s,
                             slice(None), pl.ds(col, _COMPUTE_COLS))
                            for s in range(strips_per_channel)
                            for col in range(0, width, _COMPUTE_COLS)]
                        return fn(a * channels_per_way + c, tiles, carry)
                    return lax.fori_loop(0, channels_per_way, channel, carry)
                return lax.fori_loop(0, ways_per_group, way, init)

            def average(fn):
                def add(c, tiles, acc):
                    for tile in tiles:
                        acc = acc + fn(buf[tile].astype(jnp.float32))
                    return acc
                acc = for_channels(add, jnp.zeros((_ROWS, _COMPUTE_COLS), jnp.float32))
                acc = jnp.sum(acc, axis=0, keepdims=True)
                return jnp.sum(acc, axis=1, keepdims=True) * inv_count

            before_pass(3 * k)
            mean = _splat(average(lambda v: v))
            before_pass(3 * k + 1)
            var = average(lambda v: jnp.square(v - mean))
            rstd = jnp.broadcast_to(lax.rsqrt(var + _EPS), (1, _LANES))
            before_pass(3 * k + 2)
            first_channel = channels_per_group * lax.rem(
                window * _GROUPS_PER_WINDOW + k, _GROUPS)

            def affine(c, tiles, carry):
                row = pl.ds(first_channel + c, 1)
                scale = _splat(g_tab[row, :] * rstd)
                shift = _splat(b_tab[row, :])
                for tile in tiles:
                    v = buf[tile].astype(jnp.float32)
                    buf[tile] = ((v - mean) * scale + shift).astype(buf.dtype)
            for_channels(affine)
        _loop(0, _GROUPS_PER_WINDOW, group)

    g_copy = pltpu.make_async_copy(g_hbm, g_vmem, param_sems.at[0])
    b_copy = pltpu.make_async_copy(b_hbm, b_vmem, param_sems.at[1])
    bulk = strips - _TAIL_STRIPS
    passes = 3 * _GROUPS_PER_WINDOW
    burst = bulk // passes

    def phase(p):
        lo = lax.div(p * (windows // 2), _PHASES)
        pairs = lax.div((p + 1) * (windows // 2), _PHASES) - lo
        first, last = 2 * lo, 2 * (pairs - 1)

        _loop(0, pairs - 1, lambda i: start_reads(
            first + 2 * i, 2 * i, 0, strips, read_sems.at[i]))

        @pl.when(p == 0)
        def _():
            g_copy.wait()
            b_copy.wait()
            _lane_splat_table(g_vmem, g_tab)
            _lane_splat_table(b_vmem, b_tab)

        last_sem = read_sems.at[pairs - 1]
        wait_reads(first, 0, 0, strips, read_sems.at[0])
        normalise(first, 0, lambda i: start_reads(
            first + last, last, i * burst, (i + 1) * burst, last_sem))
        if passes * burst < bulk:
            start_reads(first + last, last, passes * burst, bulk, last_sem)
        start_reads(first + last, last, bulk, strips, tail_sem)
        _loop(1, pairs - 1, lambda i: wait_reads(
            first + 2 * i, 2 * i, 0, strips, read_sems.at[i]))
        wait_reads(first + last, last, 0, bulk, last_sem)

        start_writes(first, 0)
        wait_reads(first + last, last, bulk, strips, tail_sem)

        def drain(s):
            normalise(first + s, s)
            start_writes(first + s, s)
        _loop(1, 2 * pairs, drain)
        _loop(0, 2 * pairs, lambda s: wait_writes(first + s, s))

    g_copy.start()
    b_copy.start()
    _loop(0, _PHASES, phase)


@jax.jit
def pallas_standalone__groupnorm__prompt_kernel(
    x: jax.Array,
    g: jax.Array,
    b: jax.Array,
):
    batch, channels, height, width = x.shape
    windows = batch * _GROUPS // _GROUPS_PER_WINDOW
    strips = batch * channels * (height // _ROWS) // (windows * _WAYS)
    window_shape = (_WAYS, strips, _ROWS, width)
    assert windows % 2 == 0 and windows // 2 >= 2 * _PHASES
    assert channels % (_GROUPS * _WAYS // _GROUPS_PER_WINDOW) == 0
    assert channels % _LANES == 0 and height % _ROWS == 0 and strips > _TAIL_STRIPS
    assert width % _WRITE_COLS == 0 and width % _COMPUTE_COLS == 0
    max_pairs = -(-(windows // 2) // _PHASES)

    out = pl.pallas_call(
        functools.partial(_kernel, height=height),
        in_specs=[pl.BlockSpec(memory_space=pl.ANY)] * 3,
        out_specs=pl.BlockSpec(memory_space=pl.ANY),
        out_shape=jax.ShapeDtypeStruct((windows, *window_shape), x.dtype),
        scratch_shapes=[
            pltpu.VMEM((2 * max_pairs, *window_shape), x.dtype),
            pltpu.VMEM(g.shape, g.dtype),
            pltpu.VMEM(b.shape, b.dtype),
            pltpu.VMEM((channels, _LANES), jnp.float32),
            pltpu.VMEM((channels, _LANES), jnp.float32),
            pltpu.SemaphoreType.DMA((max_pairs,)),
            pltpu.SemaphoreType.DMA,
            pltpu.SemaphoreType.DMA((2 * max_pairs,)),
            pltpu.SemaphoreType.DMA((2,)),
        ],
        compiler_params=pltpu.CompilerParams(vmem_limit_bytes=120 * 2**20),
        name="groupnorm",
    )(x.reshape(windows, *window_shape), g, b)
    return out.reshape(x.shape)
```

```python
import functools

import jax
import jax.numpy as jnp
from jax import lax
import jax.experimental.pallas as pl
import jax.experimental.pallas.tpu as pltpu

_GROUPS = 32
_EPS = 1e-5
_LANES = 128
_ROWS = 8
_WAYS = 8
_GROUPS_PER_WINDOW = 2
_READ_COLS = 256
_WRITE_COLS = 1024
_COMPUTE_COLS = 1024
_READ_TAIL = 2
_WRITE_TAIL = 1
_PHASES = 3


def _loop(lo, hi, fn):
    lax.fori_loop(lo, hi, lambda i, carry: fn(i), None)


def _lane_splat_table(v_ref, table_ref):
    n = v_ref.shape[0]
    v = v_ref[...].astype(jnp.float32).reshape(1, n)
    for c in range(0, n, _LANES):
        table_ref[c:c + _LANES, :] = jnp.broadcast_to(
            v[:, c:c + _LANES], (_LANES, _LANES)).T


def _splat(v):
    return jnp.tile(jnp.broadcast_to(v, (_ROWS, _LANES)), (1, _COMPUTE_COLS // _LANES))


def _kernel(x_hbm, g_hbm, b_hbm, o_hbm, buf, g_vmem, b_vmem, g_tab, b_tab,
            first_sem, bulk_sem, last_sem, tail_sem, param_sem, *, height):
    windows, _, strips, _, width = x_hbm.shape
    ways_per_group = _WAYS // _GROUPS_PER_WINDOW
    strips_per_channel = height // _ROWS
    channels_per_way = strips // strips_per_channel
    channels_per_group = ways_per_group * channels_per_way
    inv_count = 1.0 / (channels_per_group * height * width)

    def start_reads(window, slot, lo, hi, sem):
        def strip(s):
            for col in range(0, width, _READ_COLS):
                for thread in range(2):
                    part = (slice(None), s, slice(None), pl.ds(col, _READ_COLS))
                    pltpu.make_async_copy(
                        x_hbm.at[(window + thread, *part)],
                        buf.at[(slot + thread, *part)], sem).start(priority=thread)
        _loop(lo, hi, strip)

    def start_writes(window, slot, lo, hi, sem):
        def strip(s):
            for col in range(0, width, _WRITE_COLS):
                part = (slice(None), s, slice(None), pl.ds(col, _WRITE_COLS))
                pltpu.make_async_copy(
                    buf.at[(slot, *part)], o_hbm.at[(window, *part)], sem).start()
        _loop(lo, hi, strip)

    def wait_reads(window, slot, n, lo, hi, sem):
        pltpu.make_async_copy(
            x_hbm.at[window:window + n, :, lo:hi], buf.at[slot:slot + n, :, lo:hi],
            sem).wait()

    def wait_writes(window, slot, n, lo, hi, sem):
        pltpu.make_async_copy(
            buf.at[slot:slot + n, :, lo:hi], o_hbm.at[window:window + n, :, lo:hi],
            sem).wait()

    def normalise(window, slot, before_pass=lambda i: None):
        def group(k):
            def for_channels(fn, init=None):
                def way(a, carry):
                    def channel(c, carry):
                        tiles = [
                            (slot, k * ways_per_group + a, c * strips_per_channel + s,
                             slice(None), pl.ds(col, _COMPUTE_COLS))
                            for s in range(strips_per_channel)
                            for col in range(0, width, _COMPUTE_COLS)]
                        return fn(a * channels_per_way + c, tiles, carry)
                    return lax.fori_loop(0, channels_per_way, channel, carry)
                return lax.fori_loop(0, ways_per_group, way, init)

            def average(fn):
                def add(c, tiles, acc):
                    for tile in tiles:
                        acc = acc + fn(buf[tile].astype(jnp.float32))
                    return acc
                acc = for_channels(add, jnp.zeros((_ROWS, _COMPUTE_COLS), jnp.float32))
                acc = jnp.sum(acc, axis=0, keepdims=True)
                return jnp.sum(acc, axis=1, keepdims=True) * inv_count

            before_pass(3 * k)
            mean = _splat(average(lambda v: v))
            before_pass(3 * k + 1)
            var = average(lambda v: jnp.square(v - mean))
            rstd = jnp.broadcast_to(lax.rsqrt(var + _EPS), (1, _LANES))
            before_pass(3 * k + 2)
            first_channel = channels_per_group * lax.rem(
                window * _GROUPS_PER_WINDOW + k, _GROUPS)

            def affine(c, tiles, carry):
                row = pl.ds(first_channel + c, 1)
                scale = _splat(g_tab[row, :] * rstd)
                shift = _splat(b_tab[row, :])
                for tile in tiles:
                    v = buf[tile].astype(jnp.float32)
                    buf[tile] = ((v - mean) * scale + shift).astype(buf.dtype)
            for_channels(affine)
        _loop(0, _GROUPS_PER_WINDOW, group)

    read_bulk = strips - _READ_TAIL
    write_bulk = strips - _WRITE_TAIL
    passes = 3 * _GROUPS_PER_WINDOW
    burst = read_bulk // passes

    def phase(first, count, finish_previous):
        pair, end = count - 2, count - 1

        start_reads(first, 0, 0, strips, first_sem)
        finish_previous()
        _loop(1, pair // 2, lambda i: start_reads(
            first + 2 * i, 2 * i, 0, strips, bulk_sem))

        wait_reads(first, 0, 2, 0, strips, first_sem)
        normalise(first, 0, lambda i: start_reads(
            first + pair, pair, i * burst, (i + 1) * burst, last_sem))
        if passes * burst < read_bulk:
            start_reads(first + pair, pair, passes * burst, read_bulk, last_sem)
        start_reads(first + pair, pair, read_bulk, strips, tail_sem)
        wait_reads(first + 2, 2, pair - 2, 0, strips, bulk_sem)
        wait_reads(first + pair, pair, 2, 0, read_bulk, last_sem)

        start_writes(first, 0, 0, strips, bulk_sem)
        wait_reads(first + pair, pair, 2, read_bulk, strips, tail_sem)

        def drain(s):
            normalise(first + s, s)

            @pl.when(s < end)
            def _():
                start_writes(first + s, s, 0, strips, bulk_sem)
        _loop(1, count, drain)
        start_writes(first + end, end, 0, write_bulk, last_sem)
        start_writes(first + end, end, write_bulk, strips, tail_sem)
        wait_writes(first, 0, end, 0, strips, bulk_sem)
        wait_writes(first + end, end, 1, 0, write_bulk, last_sem)
        return lambda: wait_writes(first + end, end, 1, write_bulk, strips, tail_sem)

    g_copy = pltpu.make_async_copy(g_hbm, g_vmem, param_sem)
    b_copy = pltpu.make_async_copy(b_hbm, b_vmem, param_sem)
    g_copy.start()
    b_copy.start()

    def finish():
        g_copy.wait()
        b_copy.wait()
        _lane_splat_table(g_vmem, g_tab)
        _lane_splat_table(b_vmem, b_tab)

    bounds = [2 * (p * (windows // 2) // _PHASES) for p in range(_PHASES + 1)]
    for lo, hi in zip(bounds, bounds[1:]):
        finish = phase(lo, hi - lo, finish)
    finish()


@jax.jit
def pallas_standalone__groupnorm__prompt_kernel(
    x: jax.Array,
    g: jax.Array,
    b: jax.Array,
):
    batch, channels, height, width = x.shape
    windows = batch * _GROUPS // _GROUPS_PER_WINDOW
    strips = batch * channels * (height // _ROWS) // (windows * _WAYS)
    window_shape = (_WAYS, strips, _ROWS, width)
    assert windows % 2 == 0 and windows // 2 >= 3 * _PHASES
    assert channels % (_GROUPS * _WAYS // _GROUPS_PER_WINDOW) == 0
    assert channels % _LANES == 0 and height % _ROWS == 0 and strips > _READ_TAIL
    assert width % _WRITE_COLS == 0 and width % _COMPUTE_COLS == 0
    max_pairs = -(-(windows // 2) // _PHASES)

    out = pl.pallas_call(
        functools.partial(_kernel, height=height),
        in_specs=[pl.BlockSpec(memory_space=pl.ANY)] * 3,
        out_specs=pl.BlockSpec(memory_space=pl.ANY),
        out_shape=jax.ShapeDtypeStruct((windows, *window_shape), x.dtype),
        scratch_shapes=[
            pltpu.VMEM((2 * max_pairs, *window_shape), x.dtype),
            pltpu.VMEM(g.shape, g.dtype),
            pltpu.VMEM(b.shape, b.dtype),
            pltpu.VMEM((channels, _LANES), jnp.float32),
            pltpu.VMEM((channels, _LANES), jnp.float32),
            *[pltpu.SemaphoreType.DMA] * 5,
        ],
        compiler_params=pltpu.CompilerParams(vmem_limit_bytes=120 * 2**20),
        name="groupnorm",
    )(x.reshape(windows, *window_shape), g, b)
    return out.reshape(x.shape)
```
